```python
import jax
import jax.numpy as jnp

def _softmax(x, axis=-1):
    return jax.nn.softmax(x, axis=axis)
def _gelu(x):
    return jax.nn.gelu(x, approximate=True)
def _silu(x):
    return jax.nn.silu(x)
def _sigmoid(x):
    return jax.nn.sigmoid(x)
def _layernorm(x, axis=-1, eps=1e-5):
    m = jnp.mean(x, axis=axis, keepdims=True)
    v = jnp.var(x, axis=axis, keepdims=True)
    return (x - m) / jnp.sqrt(v + eps)
def _scatter_add(tgt, idx, src, axis=0):
    return tgt.at[idx].add(src)
def _segment_sum(src, seg, n):
    return jax.ops.segment_sum(src, seg, n)
class _Rng:
    def __init__(self, key):
        self._k = key
    def _next(self):
        self._k, sub = jax.random.split(self._k)
        return sub
    def normal(self, shape):
        return jax.random.normal(self._next(), shape, dtype=jnp.bfloat16)
    def randint(self, lo, hi, shape):
        return jax.random.randint(self._next(), shape, lo, hi, dtype=jnp.int32)
    def uniform(self, shape, lo=0.0, hi=1.0):
        return jax.random.uniform(self._next(), shape, jnp.bfloat16, lo, hi)
    def permutation(self, n):
        return jax.random.permutation(self._next(), n)


kernel_name = 'standalone__modern_conv_block_convnext__vision'

def setup_inputs():
    _rng = _Rng(jax.random.key(int.from_bytes(__import__("os").urandom(4), "little")))
    _w = (lambda a: (lambda t: t.astype(jnp.bfloat16) if jnp.issubdtype(t.dtype, jnp.floating) else t)(jnp.asarray(a)))
    H = W = 512
    C = 96
    K = 3
    return {
        "x": _w((lambda *s: _rng.normal(s) * 0.05)(1, H, W, C)),
        "dw": _w((lambda *s: _rng.normal(s) * 0.05)(K, K, C)),
        "w1": _w((lambda *s: _rng.normal(s) * 0.05)(C, 4 * C)),
        "b1": _w((lambda *s: _rng.normal(s) * 0.05)(4 * C)),
        "w2": _w((lambda *s: _rng.normal(s) * 0.05)(4 * C, C)),
        "b2": _w((lambda *s: _rng.normal(s) * 0.05)(C)),
        "gamma": _w((lambda *s: _rng.normal(s) * 0.05)(C)),
    }

def reference(x, dw, w1, b1, w2, b2, gamma):
    B, H, W, C = x.shape
    K = dw.shape[0]
    pad = K // 2
    xp = jnp.pad(x, ((0,0),(pad,pad),(pad,pad),(0,0)))
    out = jnp.zeros_like(x)
    for i in range(K):
        for j in range(K):
            out = out + xp[:, i:i+H, j:j+W, :] * dw[i, j][None, None, None, :]
    h = _layernorm(out, axis=-1)
    h = jnp.einsum('bhwc,ce->bhwe', h, w1) + b1
    h = _gelu(h)
    h = jnp.einsum('bhwe,ec->bhwc', h, w2) + b2
    return x + gamma[None, None, None, :] * h
```

```python
import functools
import jax, jax.numpy as jnp
from jax import lax
import jax.experimental.pallas as pl
import jax.experimental.pallas.tpu as pltpu

H = W = 512; C = 96; E = 384
F32 = jnp.float32; BF16 = jnp.bfloat16
GA = 0.7978845608028654; GB = 0.044715
S3 = (GA * GB) ** (1.0 / 3.0)
A1 = GA / S3

def col(v):
    n = v.shape[-1]
    return jnp.broadcast_to(v, (128, n)).T

def pallas_standalone__modern_conv_block_convnext__vision_kernel(x, dw, w1, b1, w2, b2, gamma, TH=8):
    xt = jnp.transpose(x, (0, 1, 3, 2)).reshape(H, C, W)
    w2t = w2.T
    nb = H // TH

    def body(xp_ref, x_ref, xn_ref, dw_ref, w1_ref, b1_ref, w2_ref, b2_ref, g_ref, o_ref, dws, w1s, w2s, gbs):
        i = pl.program_id(0)

        @pl.when(i == 0)
        def _():
            pad = lambda v: jnp.concatenate([v, jnp.zeros((v.shape[0], 128 - v.shape[1]), v.dtype)], axis=1)
            for a in range(3):
                d = pad(dw_ref[a].astype(F32))
                for b in range(3):
                    dws[a * 3 + b] = col(d[b:b + 1])[:C]
            gam = col(pad(g_ref[...].astype(F32)))[:C]
            gbs[...] = gam * col(pad(b2_ref[...].astype(F32)))[:C]
            bb = b1_ref[...].astype(F32) * S3
            w1f = jnp.concatenate([w1_ref[...].astype(F32), jnp.zeros((32, E), F32)], axis=0)
            row = lax.broadcasted_iota(jnp.int32, (128, E), 0)
            hi = bb.astype(BF16).astype(F32)
            w1f = jnp.where(row == C, hi, jnp.where(row == C + 1, bb - hi, w1f))
            w1s[...] = pltpu.bitcast(w1f.T.astype(BF16), jnp.uint32)
            w2f = w2_ref[...].astype(F32) * jnp.concatenate([gam] * 3, axis=1) * (0.5 / S3)
            w2s[...] = pltpu.bitcast(w2f.astype(BF16), jnp.uint32)

        top = jnp.where(i > 0, 1.0, 0.0)
        bot = jnp.where(i < nb - 1, 1.0, 0.0)
        rows = [xp_ref[0].astype(F32) * top] + [x_ref[r].astype(F32) for r in range(TH)] + [xn_ref[0].astype(F32) * bot]
        lane = lax.broadcasted_iota(jnp.int32, (C, W), 1)
        rep = lambda v: jnp.concatenate([v] * 4, axis=1)
        for r in range(TH):
            s = []
            for b in range(3):
                s.append(rows[r] * rep(dws[b]) + rows[r + 1] * rep(dws[3 + b]) + rows[r + 2] * rep(dws[6 + b]))
            sl = jnp.where(lane == 0, 0.0, pltpu.roll(s[0], 1, 1))
            sr = jnp.where(lane == W - 1, 0.0, pltpu.roll(s[2], W - 1, 1))
            y = s[1] + sl + sr
            m = jnp.mean(y, axis=0, keepdims=True)
            d = y - m
            v = jnp.mean(d * d, axis=0, keepdims=True)
            yn = d * (lax.rsqrt(v + 1e-5) * S3)
            yy = jnp.concatenate([yn, jnp.ones((32, W), F32)], axis=0)
            z = lax.dot_general(pltpu.bitcast(w1s[...], BF16), yy, (((1,), (0,)), ((), ())), preferred_element_type=F32)
            t = jnp.tanh(z * (z * z + A1))
            g = z + z * t
            o = lax.dot_general(pltpu.bitcast(w2s[...], BF16), g, (((1,), (0,)), ((), ())), preferred_element_type=F32)
            o_ref[r] = (o + rep(gbs[...]) + rows[r + 1]).astype(BF16)

    full = lambda s: pl.BlockSpec(s, lambda i: (0,) * len(s))
    out = pl.pallas_call(body, grid=(nb,),
        in_specs=[pl.BlockSpec((1, C, W), lambda i: (jnp.maximum(i * TH - 1, 0), 0, 0)),
                  pl.BlockSpec((TH, C, W), lambda i: (i, 0, 0)),
                  pl.BlockSpec((1, C, W), lambda i: (jnp.minimum(i * TH + TH, H - 1), 0, 0)),
                  full((3, 3, C)), full((C, E)), full((1, E)), full((C, E)), full((1, C)), full((1, C))],
        out_specs=pl.BlockSpec((TH, C, W), lambda i: (i, 0, 0)),
        scratch_shapes=[pltpu.VMEM((9, C, 128), F32), pltpu.VMEM((E // 2, 128), jnp.uint32), pltpu.VMEM((C // 2, E), jnp.uint32), pltpu.VMEM((C, 128), F32)],
        out_shape=jax.ShapeDtypeStruct((H, C, W), BF16),
        compiler_params=pltpu.CompilerParams(dimension_semantics=("arbitrary",), vmem_limit_bytes=100 * 1024 * 1024),
    )(xt, xt, xt, dw, w1, b1.reshape(1, E), w2t, b2.reshape(1, C), gamma.reshape(1, C))
    return jnp.transpose(out.reshape(1, H, W, C) if False else out.reshape(1, H, C, W), (0, 1, 3, 2))
```

```python
import functools
import jax, jax.numpy as jnp
from jax import lax
import jax.experimental.pallas as pl
import jax.experimental.pallas.tpu as pltpu

H = W = 512; C = 96; E = 384
F32 = jnp.float32; BF16 = jnp.bfloat16; U32 = jnp.uint32
EPS = 1e-5
GA = 0.7978845608028654; GB = 0.044715
S3 = (GA * GB) ** (1.0 / 3.0)
A1 = GA / S3
NG = C // 8


def dot(a, b):
    return lax.dot_general(a, b, (((1,), (0,)), ((), ())), preferred_element_type=F32)


def col(v):
    return jnp.broadcast_to(v, (128, 128)).T


def pallas_standalone__modern_conv_block_convnext__vision_kernel(x, dw, w1, b1, w2, b2, gamma, U=15, order='BdbAc', f32g=True, flags=()):
    xt = jnp.transpose(x, (0, 1, 3, 2)).reshape(H, C, W)
    w2t = w2.T
    R0 = 2
    NI = (H - R0) // U
    assert R0 + NI * U == H

    def body(x_hbm, dw_ref, w1_ref, b1_ref, w2_ref, b2_ref, g_ref, o_hbm,
             xp, xb, ob, oe, dws, w1s, w2s, cx, cy, cg, ca, sem):
        def in_copy(i, slot, n=U):
            return pltpu.make_async_copy(x_hbm.at[pl.ds(R0 + 1 + i * U, n)], xb.at[slot, pl.ds(0, n)], sem.at[slot])
        def out_copy(i, slot):
            return pltpu.make_async_copy(ob.at[slot], o_hbm.at[pl.ds(i * U, U)], sem.at[2 + slot])
        pro_copy = pltpu.make_async_copy(x_hbm.at[pl.ds(0, R0 + 1)], xp, sem.at[4])
        epi_copy = pltpu.make_async_copy(oe, o_hbm.at[pl.ds(H - 2, 2)], sem.at[5])
        pro_copy.start()
        in_copy(0, 0).start()

        pad = lambda v: jnp.concatenate([v, jnp.zeros((v.shape[0], 128 - v.shape[1]), v.dtype)], axis=1)
        for a in range(3):
            d = pad(dw_ref[a].astype(F32))
            for b in range(3):
                dws[a * 3 + b] = col(d[b:b + 1])[:C]
        gam = col(pad(g_ref[...].astype(F32)))[:C]
        dws[9] = gam * col(pad(b2_ref[...].astype(F32)))[:C]
        bb = b1_ref[...].astype(F32) * S3
        w1f = w1_ref[...].astype(F32)
        w1f = w1f - jnp.mean(w1f, axis=0, keepdims=True)
        w1f = jnp.concatenate([w1f, jnp.zeros((128 - C, E), F32)], axis=0)
        row = lax.broadcasted_iota(jnp.int32, (128, E), 0)
        hi = bb.astype(BF16).astype(F32)
        w1f = jnp.where(row == C, hi, jnp.where(row == C + 1, bb - hi, w1f))
        w1f = w1f.T
        w1f = jnp.concatenate([w1f[128 * (i // 16) + 8 * (15 - i % 16):][:8] for i in range(E // 8)], axis=0)
        w1s[...] = pltpu.bitcast(w1f.astype(BF16), U32)
        w2f = w2_ref[...].astype(F32) * jnp.concatenate([gam] * 3, axis=1) * (0.5 / S3)
        w2s[...] = pltpu.bitcast(w2f.astype(BF16), U32)

        sub = lax.broadcasted_iota(jnp.int32, (8, 128), 0)
        lane = lax.broadcasted_iota(jnp.int32, (8, W), 1)
        rep = lambda v: jnp.concatenate([v] * 4, axis=1)
        hs = lambda h: slice(256 * h, 256 * (h + 1))
        G8 = lambda k: slice(8 * k, 8 * k + 8)

        def emit(r0, r1, xsrc, odst, first, last):
            X = {}; Y = {}; YN = {}; G = {}; ACC = {}; ST = {}

            def getx(r, k):
                if (r, k) not in X:
                    if r < 0: return None
                    if first or r > r0:
                        v = xsrc(r, k // 2).astype(F32)
                        X[r, k // 2 * 2] = v[:8]; X[r, k // 2 * 2 + 1] = v[8:]
                    else:
                        return cx[r - r0 + 1, G8(k), :]
                return X[r, k]

            def conv(r, k):
                xs = [getx(r - 1 + i, k) for i in range(3)]
                s = []
                for b in range(3):
                    t = None
                    for i in range(3):
                        if xs[i] is None: continue
                        p = xs[i] * rep(dws[3 * i + b, G8(k), :])
                        t = p if t is None else t + p
                    s.append(t)
                l = jnp.where(lane == 0, 0.0, pltpu.roll(s[0], 1, 1))
                rr = jnp.where(lane == W - 1, 0.0, pltpu.roll(s[2], W - 1, 1))
                y = s[1] + l + rr
                Y[r, k] = y
                ST[r] = (y, y * y) if k == 0 else (ST[r][0] + y, ST[r][1] + y * y)

            def bfly(v):
                t = [v[:, 128 * j:128 * j + 128] for j in range(4)]
                h4 = sub < 4; h2 = (sub & 2) == 0
                u = [jnp.where(h4, t[2 * i], t[2 * i + 1]) + pltpu.roll(jnp.where(h4, t[2 * i + 1], t[2 * i]), 4, 0) for i in range(2)]
                w = jnp.where(h2, u[1] + pltpu.roll(u[1], 6, 0), u[0] + pltpu.roll(u[0], 2, 0))
                return w + pltpu.roll(w, 1, 0)

            def norm(r):
                m = bfly(ST[r][0]) * (1.0 / C)
                v = jnp.maximum(bfly(ST[r][1]) * (1.0 / C) - m * m, 0.0)
                rs = lax.rsqrt(v + EPS) * S3
                rs = jnp.concatenate([jnp.broadcast_to(rs[i:i + 1], (8, 128)) for i in (3, 7, 1, 5)], axis=1)
                YN[r] = [Y.pop((r, k)) * rs for k in range(NG)]

            def up(m, h):
                r, kk = divmod(m, 3)
                if r in YN: yy = jnp.concatenate([v[:, hs(h)] for v in YN[r]], axis=0)
                else: yy = cy[:, hs(h)]
                yy = jnp.concatenate([yy, jnp.ones((128 - C, 256), F32)], axis=0)
                z = dot(pltpu.bitcast(w1s[64 * kk:64 * kk + 64, :], BF16), yy)
                t = jnp.tanh(z * (z * z + A1))
                g = z + z * t
                G[m, h] = jnp.concatenate([g[G8(i)] for i in reversed(range(16))], axis=0)

            def down(q, h):
                r, kk = divmod(q, 3)
                g = G.pop((q, h)) if (q, h) in G else cg[1 + q - (3 * r0 - 5) if h else 0]
                if not f32g: g = g.astype(BF16)
                o = dot(pltpu.bitcast(w2s[:, 128 * kk:128 * kk + 128], BF16), g)
                if kk == 0:
                    o = o + jnp.concatenate([dws[9, G8(k), :][:, None, :].reshape(8, 128) for k in range(0)] + [jnp.concatenate([dws[9, G8(k), :]] * 2, axis=1) + (X[r, k][:, hs(h)] if (r, k) in X else cx[r - r0 + 1, G8(k), hs(h)]) for k in range(NG)], axis=0)
                else:
                    o = o + (ACC.pop(h) if h in ACC else ca[:, hs(h)])
                if kk == 2: odst(r, h, o.astype(BF16))
                else: ACC[h] = o

            for n in range(3 * r0, 3 * r1 + (5 if last else 0)):
                r, kk = divmod(n, 3)
                ok = lambda j: 0 <= j < 3 * r1
                for c in order:
                    if c == 'A' and r < r1:
                        for k in range(4 * kk, 4 * kk + 4): conv(r, k)
                        if kk == 2: norm(r)
                    if c == 'B' and ok(n - 3): up(n - 3, 0)
                    if c == 'b' and ok(n - 3): up(n - 3, 1)
                    if c == 'c' and ok(n - 4): down(n - 4, 0)
                    if c == 'd' and ok(n - 5): down(n - 5, 1)
            if not last:
                for i in range(2):
                    for k in range(NG): cx[i, G8(k), :] = X[r1 - 1 + i, k]
                for k in range(NG): cy[G8(k), :] = YN[r1 - 1][k]
                for (q, h), v in G.items(): cg[1 + q - (3 * r1 - 5) if h else 0] = v
                for h, v in ACC.items(): ca[:, hs(h)] = v

        in_copy(1, 1).start()
        pro_copy.wait()
        emit(0, R0, lambda r, p: xp[r, 16 * p:16 * p + 16, :], None, True, False)

        def step(i, carry):
            slot = i % 2
            @pl.when(i < NI - 1)
            def _():
                in_copy(i, slot).wait()
            @pl.when(i == NI - 1)
            def _():
                in_copy(i, slot, U - 1).wait()
                xb[slot, U - 1] = jnp.zeros((C, W), BF16)
            @pl.when(i >= 2)
            def _():
                out_copy(i - 2, slot).wait()
            def odst(r, h, v): ob[slot, r, :, hs(h)] = v
            emit(R0, R0 + U, lambda r, p: xb[slot, r - R0 - 1, 16 * p:16 * p + 16, :], odst, False, False)
            out_copy(i, slot).start()
            @pl.when(i + 2 < NI - 1)
            def _():
                in_copy(i + 2, slot).start()
            @pl.when(i + 2 == NI - 1)
            def _():
                in_copy(i + 2, slot, U - 1).start()
            return carry
        lax.fori_loop(0, NI, step, 0)

        def odst(r, h, v): oe[r - (R0 + U - 2), :, hs(h)] = v
        emit(R0 + U, R0 + U, None, odst, False, True)
        epi_copy.start()
        out_copy(NI - 2, (NI - 2) % 2).wait()
        out_copy(NI - 1, (NI - 1) % 2).wait()
        epi_copy.wait()

    V = pltpu.VMEM
    vm = pl.BlockSpec(memory_space=V)
    out = pl.pallas_call(
        body,
        in_specs=[pl.BlockSpec(memory_space=pl.ANY)] + [vm] * 6,
        out_specs=pl.BlockSpec(memory_space=pl.ANY),
        scratch_shapes=[V((R0 + 1, C, W), BF16), V((2, U, C, W), BF16), V((2, U, C, W), BF16), V((2, C, W), BF16),
                        V((10, C, 128), F32), V((E // 2, 128), U32), V((C // 2, E), U32),
                        V((2, C, W), F32), V((C, W), F32), V((3, 128, 256), F32), V((C, W), F32),
                        pltpu.SemaphoreType.DMA((6,))],
        out_shape=jax.ShapeDtypeStruct((H, C, W), BF16),
        compiler_params=pltpu.CompilerParams(vmem_limit_bytes=100 * 1024 * 1024, flags={f: True for f in flags}),
    )(xt, dw, w1, b1.reshape(1, E), w2t, b2.reshape(1, C), gamma.reshape(1, C))
    return jnp.transpose(out.reshape(1, H, C, W), (0, 1, 3, 2))
```

```python
import functools
import jax, jax.numpy as jnp
from jax import lax
import jax.experimental.pallas as pl
import jax.experimental.pallas.tpu as pltpu

H = W = 512; C = 96; E = 384
F32 = jnp.float32; BF16 = jnp.bfloat16; U32 = jnp.uint32
EPS = 1e-5
GA = 0.7978845608028654; GB = 0.044715
S3 = (GA * GB) ** (1.0 / 3.0)
A1 = GA / S3
NG = C // 8


def dot(a, b):
    return lax.dot_general(a, b, (((1,), (0,)), ((), ())), preferred_element_type=F32)


def col(v):
    return jnp.broadcast_to(v, (128, 128)).T


def pallas_standalone__modern_conv_block_convnext__vision_kernel(x, dw, w1, b1, w2, b2, gamma):
    return _block(x, dw, w1, b1, w2, b2, gamma)


pallas_standalone__modern_conv_block_convnext__vision_kernel = jax.jit(pallas_standalone__modern_conv_block_convnext__vision_kernel)


def _block(x, dw, w1, b1, w2, b2, gamma, U=28, R0=8, osp=24, oc=6, order='BdcbA'):
    xt = jnp.transpose(x, (0, 1, 3, 2)).reshape(H, C, W)
    w2t = w2.T
    NI = (H - R0) // U
    assert R0 + NI * U == H

    def body(x_hbm, dw_ref, w1_ref, b1_ref, w2_ref, b2_ref, g_ref, o_hbm,
             xp, xb, ob, oe, op, dws, w1s, w2s, cx, cy, cg, ca, sem):
        def in_copy(i, slot):
            st = jnp.minimum(R0 + 1 + i * U, H - U)
            return pltpu.make_async_copy(x_hbm.at[pl.ds(st, U)], xb.at[slot, pl.ds(0, U)], sem.at[slot])
        NP = R0 - 2
        po_copy = pltpu.make_async_copy(op, o_hbm.at[pl.ds(0, NP)], sem.at[6])
        def out_copy(i, slot, a=0, b=U):
            return pltpu.make_async_copy(ob.at[slot, pl.ds(a, b - a)], o_hbm.at[pl.ds(R0 - 2 + i * U + a, b - a)], sem.at[2 + slot])
        pro_copy = pltpu.make_async_copy(x_hbm.at[pl.ds(0, R0 + 1)], xp, sem.at[4])
        epi_copy = pltpu.make_async_copy(oe, o_hbm.at[pl.ds(H - 2, 2)], sem.at[5])
        pro_copy.start()
        in_copy(0, 0).start()

        pad = lambda v: jnp.concatenate([v, jnp.zeros((v.shape[0], 128 - v.shape[1]), v.dtype)], axis=1)
        for a in range(3):
            d = pad(dw_ref[a].astype(F32))
            for b in range(3):
                dws[a * 3 + b] = col(d[b:b + 1])[:C]
        gam = col(pad(g_ref[...].astype(F32)))[:C]
        dws[9] = gam * col(pad(b2_ref[...].astype(F32)))[:C]
        bb = b1_ref[...].astype(F32).reshape(1, E) * S3
        w1f = w1_ref[...].astype(F32)
        w1f = w1f - jnp.mean(w1f, axis=0, keepdims=True)
        w1f = jnp.concatenate([w1f, jnp.zeros((128 - C, E), F32)], axis=0)
        row = lax.broadcasted_iota(jnp.int32, (128, E), 0)
        hi = bb.astype(BF16).astype(F32)
        w1f = jnp.where(row == C, hi, jnp.where(row == C + 1, bb - hi, w1f))
        w1f = w1f.T
        w1f = jnp.concatenate([w1f[128 * (i // 16) + 8 * (15 - i % 16):][:8] for i in range(E // 8)], axis=0)
        w1s[...] = pltpu.bitcast(w1f.astype(BF16), U32)
        w2f = w2_ref[...].astype(F32) * jnp.concatenate([gam] * 3, axis=1) * (0.5 / S3)
        w2s[...] = pltpu.bitcast(w2f.astype(BF16), U32)

        sub = lax.broadcasted_iota(jnp.int32, (8, 128), 0)
        lane = lax.broadcasted_iota(jnp.int32, (8, W), 1)
        rep = lambda v: jnp.concatenate([v] * 4, axis=1)
        hs = lambda h: slice(256 * h, 256 * (h + 1))
        G8 = lambda k: slice(8 * k, 8 * k + 8)

        def emit(r0, r1, xsrc, odst, first, last):
            X = {}; Y = {}; YN = {}; G = {}; ACC = {}; ST = {}

            def getx(r, k):
                if (r, k) not in X:
                    if r < 0: return None
                    if first or r > r0:
                        v = xsrc(r, k // 2).astype(F32)
                        X[r, k // 2 * 2] = v[:8]; X[r, k // 2 * 2 + 1] = v[8:]
                    else:
                        return cx[r - r0 + 2, G8(k), :]
                return X[r, k]

            def conv(r, k):
                xs = [getx(r - 1 + i, k) for i in range(3)]
                taps = lambda b: [xs[i] * rep(dws[3 * i + b, G8(k), :]) for i in range(3) if xs[i] is not None]
                side = []
                for b in (0, 2):
                    p = taps(b)
                    t = p[0]
                    for q in p[1:]: t = t + q
                    side.append(t)
                l = jnp.where(lane == 0, 0.0, pltpu.roll(side[0], 1, 1))
                rr = jnp.where(lane == W - 1, 0.0, pltpu.roll(side[1], W - 1, 1))
                y = l + rr
                for p in taps(1): y = y + p
                Y[r, k] = y
                ST[r] = (y, y * y) if k == 0 else (ST[r][0] + y, ST[r][1] + y * y)

            def bfly(v):
                t = [v[:, 128 * j:128 * j + 128] for j in range(4)]
                h4 = sub < 4; h2 = (sub & 2) == 0
                u = [jnp.where(h4, t[2 * i], t[2 * i + 1]) + pltpu.roll(jnp.where(h4, t[2 * i + 1], t[2 * i]), 4, 0) for i in range(2)]
                w = jnp.where(h2, u[1] + pltpu.roll(u[1], 6, 0), u[0] + pltpu.roll(u[0], 2, 0))
                return w + pltpu.roll(w, 1, 0)

            def norm(r):
                m = bfly(ST[r][0]) * (1.0 / C)
                v = jnp.maximum(bfly(ST[r][1]) * (1.0 / C) - m * m, 0.0)
                rs = lax.rsqrt(v + EPS) * S3
                rs = jnp.concatenate([jnp.broadcast_to(rs[i:i + 1], (8, 128)) for i in (3, 7, 1, 5)], axis=1)
                YN[r] = [Y.pop((r, k)) * rs for k in range(NG)]

            def up(m, h):
                r, kk = divmod(m, 3)
                if r in YN: yy = jnp.concatenate([v[:, hs(h)] for v in YN[r]], axis=0)
                else: yy = cy[:, hs(h)]
                one = jnp.ones((8, 256), F32)
                if h == 0 and m + 1 in Q:
                    s2 = Q[m + 1]
                    neg = s2[:, 0:128] < -1.0
                    for j in range(1, 4): neg = neg | (s2[:, 128 * j:128 * j + 128] < -1.0)
                    one = jnp.concatenate([jnp.where(neg, 0.0, 1.0), one[:, :128]], axis=1)
                yy = jnp.concatenate([yy, jnp.ones((24, 256), F32), one], axis=0)
                z = dot(pltpu.bitcast(w1s[64 * kk:64 * kk + 64, :], BF16), yy)
                t = jnp.tanh(z * (z * z + A1))
                g = z * (t + 1.0)
                G[m, h] = jnp.concatenate([g[G8(i)] for i in reversed(range(16))], axis=0)

            def down(q, h):
                r, kk = divmod(q, 3)
                g = G.pop((q, h)) if (q, h) in G else cg[1 + q - (3 * r0 - 5) if h else 0]
                o = dot(pltpu.bitcast(w2s[:, 128 * kk:128 * kk + 128], BF16), g)
                if kk > 0: o = o + (ACC.pop(h) if h in ACC else ca[:, hs(h)])
                if kk == 2:
                    o = o + jnp.concatenate([dws[9]] * 2, axis=1)
                    o = o + jnp.concatenate([(X[r, k][:, hs(h)] if (r, k) in X else cx[r - r0 + 2, G8(k), hs(h)]) for k in range(NG)], axis=0)
                if kk == 2: odst(r, h, o.astype(BF16))
                else: ACC[h] = o

            Q = {}
            for n in range(3 * r0, 3 * r1 + (5 if last else 0)):
                r, kk = divmod(n, 3)
                ok = lambda j: 0 <= j < 3 * r1
                for c in order:
                    if c == 'A' and r < r1:
                        for k in range(4 * kk, 4 * kk + 4):
                            conv(r, k)
                            if k % 4 == 3: Q[n] = ST[r][1]
                        if kk == 2: norm(r)
                    if c == 'B' and ok(n - 3): up(n - 3, 0)
                    if c == 'b' and ok(n - 3): up(n - 3, 1)
                    if c == 'c' and ok(n - 4): down(n - 4, 0)
                    if c == 'd' and ok(n - 5): down(n - 5, 1)
            if not last:
                for i in range(3):
                    for k in range(NG): cx[i, G8(k), :] = X[r1 - 2 + i, k]
                cy[...] = jnp.concatenate(YN[r1 - 1], axis=0).astype(F32)
                for (q, h), v in G.items(): cg[1 + q - (3 * r1 - 5) if h else 0] = v
                for h, v in ACC.items(): ca[:, hs(h)] = v

        for q in range(2): xb[q, U] = jnp.zeros((C, W), BF16)
        pro_copy.wait()
        def pdst(r, h, v): op[r, :, hs(h)] = v
        emit(0, R0, lambda r, p: xp[r, 16 * p:16 * p + 16, :], pdst, True, False)
        po_copy.start()

        def step(i, carry):
            slot = i % 2
            @pl.when(i < NI - 1)
            def _():
                in_copy(i + 1, 1 - slot).start()
            in_copy(i, slot).wait()
            dl = jnp.where(i == NI - 1, 1, 0)
            def xsrc(r, p):
                j = r - R0 - 1
                return xb[slot, j + dl, 16 * p:16 * p + 16, :]
            @pl.when(i >= 2)
            def _():
                out_copy(i - 2, slot).wait()
            def odst(r, h, v):
                r = r - (R0 - 2)
                ob[slot, r, :, hs(h)] = v
                if h == 1 and r < osp and (r + 1) % oc == 0: out_copy(i, slot, r + 1 - oc, r + 1).start()
            emit(R0, R0 + U, xsrc, odst, False, False)
            out_copy(i, slot, osp, U).start()
            return carry
        lax.fori_loop(0, NI, step, 0)

        def odst(r, h, v): oe[r - (R0 + U - 2), :, hs(h)] = v
        emit(R0 + U, R0 + U, None, odst, False, True)
        epi_copy.start()
        out_copy(NI - 2, (NI - 2) % 2).wait()
        out_copy(NI - 1, (NI - 1) % 2).wait()
        epi_copy.wait()
        po_copy.wait()

    V = pltpu.VMEM
    vm = pl.BlockSpec(memory_space=V)
    out = pl.pallas_call(
        body,
        in_specs=[pl.BlockSpec(memory_space=pl.ANY)] + [vm] * 6,
        out_specs=pl.BlockSpec(memory_space=pl.ANY),
        scratch_shapes=[V((R0 + 1, C, W), BF16), V((2, U + 1, C, W), BF16), V((2, U, C, W), BF16), V((2, C, W), BF16), V((R0 - 2, C, W), BF16),
                        V((10, C, 128), F32), V((E // 2, 128), U32), V((C // 2, E), U32),
                        V((3, C, W), F32), V((C, W), F32), V((3, 128, 256), F32), V((C, W), F32),
                        pltpu.SemaphoreType.DMA((7,))],
        out_shape=jax.ShapeDtypeStruct((H, C, W), BF16),
        compiler_params=pltpu.CompilerParams(vmem_limit_bytes=100 * 1024 * 1024),
    )(xt, dw, w1, b1, w2t, b2.reshape(1, C), gamma.reshape(1, C))
    return jnp.transpose(out.reshape(1, H, C, W), (0, 1, 3, 2))
```
